```python
import os as _os
_os.environ.setdefault("JAX_PLATFORMS", "cpu")
import jax
import jax.numpy as jnp

def _softmax(x, axis=-1):
    return jax.nn.softmax(x, axis=axis)
def _gelu(x):
    return jax.nn.gelu(x, approximate=True)
def _silu(x):
    return jax.nn.silu(x)
def _sigmoid(x):
    return jax.nn.sigmoid(x)
def _layernorm(x, axis=-1, eps=1e-5):
    m = jnp.mean(x, axis=axis, keepdims=True)
    v = jnp.var(x, axis=axis, keepdims=True)
    return (x - m) / jnp.sqrt(v + eps)
def _scatter_add(tgt, idx, src, axis=0):
    return tgt.at[idx].add(src)
def _segment_sum(src, seg, n):
    return jax.ops.segment_sum(src, seg, n)
class _Rng:
    def __init__(self, key):
        self._k = key
    def _next(self):
        self._k, sub = jax.random.split(self._k)
        return sub
    def normal(self, shape):
        return jax.random.normal(self._next(), shape, dtype=jnp.bfloat16)
    def randint(self, lo, hi, shape):
        return jax.random.randint(self._next(), shape, lo, hi, dtype=jnp.int32)
    def uniform(self, shape, lo=0.0, hi=1.0):
        return jax.random.uniform(self._next(), shape, jnp.bfloat16, lo, hi)
    def permutation(self, n):
        return jax.random.permutation(self._next(), n)


kernel_name = 'concat_heads__mha_block_cached__mha_block_cached__near_ridge'

def setup_inputs():
    _rng = _Rng(jax.random.key(int.from_bytes(__import__("os").urandom(4), "little")))
    _w = (lambda a: (lambda t: t.astype(jnp.bfloat16) if jnp.issubdtype(t.dtype, jnp.floating) else t)(jnp.asarray(a)))
    def _A_setup():
        B, Sq, D = 8, 144, 640
        H, Sk, Dh = 32, 512, 128
        return {
            "x": _w((lambda *s: _rng.normal(s) * 0.8)(B, Sq, D)),
            "k_cache": _w((lambda *s: _rng.normal(s) * 0.8)(B, H, Sk, Dh)),
            "v_cache": _w((lambda *s: _rng.normal(s) * 0.05)(B, H, Sk, Dh)),
            "wq": _w((lambda *s: _rng.normal(s) * 0.8)(D, H * Dh) * (D ** -0.5)),
            "wo": _w((lambda *s: _rng.normal(s) * 0.05)(H * Dh, D) * ((H * Dh) ** -0.5)),
        }
    _A_in = _A_setup()

    def _B_setup():
        B, Sq, D = 8, 144, 640
        H, Sk, Dh = 32, 512, 128
        return {
            "x": _w((lambda *s: _rng.normal(s) * 0.8)(B, Sq, D)),
            "k_cache": _w((lambda *s: _rng.normal(s) * 0.8)(B, H, Sk, Dh)),
            "v_cache": _w((lambda *s: _rng.normal(s) * 0.05)(B, H, Sk, Dh)),
            "wq": _w((lambda *s: _rng.normal(s) * 0.8)(D, H * Dh) * (D ** -0.5)),
            "wo": _w((lambda *s: _rng.normal(s) * 0.05)(H * Dh, D) * ((H * Dh) ** -0.5)),
        }
    _B_in = _B_setup()

    return {
        "A_x": _A_in["x"],
        "A_k_cache": _A_in["k_cache"],
        "A_v_cache": _A_in["v_cache"],
        "A_wq": _A_in["wq"],
        "A_wo": _A_in["wo"],
        "B_x": _B_in["x"],
        "B_k_cache": _B_in["k_cache"],
        "B_v_cache": _B_in["v_cache"],
        "B_wq": _B_in["wq"],
        "B_wo": _B_in["wo"],
    }

def reference(A_x, A_k_cache, A_v_cache, A_wq, A_wo, B_x, B_k_cache, B_v_cache, B_wq, B_wo):
    def _A_ref(x, k_cache, v_cache, wq, wo):
        B, Sq, D = x.shape
        H, Dh = 32, 128
        q = (lambda x, *d: x.transpose(*d))((x @ wq).reshape(B, Sq, H, Dh), 0, 2, 1, 3)
        scores = jnp.einsum("bhqd,bhkd->bhqk", q, k_cache) * (Dh ** -0.5)
        p = _softmax(scores, axis=-1)
        o = jnp.einsum("bhqk,bhkd->bhqd", p, v_cache)
        return (lambda x, *d: x.transpose(*d))(o, 0, 2, 1, 3).reshape(B, Sq, H * Dh) @ wo

    def _B_ref(x, k_cache, v_cache, wq, wo):
        B, Sq, D = x.shape
        H, Dh = 32, 128
        q = (lambda x, *d: x.transpose(*d))((x @ wq).reshape(B, Sq, H, Dh), 0, 2, 1, 3)
        scores = jnp.einsum("bhqd,bhkd->bhqk", q, k_cache) * (Dh ** -0.5)
        p = _softmax(scores, axis=-1)
        o = jnp.einsum("bhqk,bhkd->bhqd", p, v_cache)
        return (lambda x, *d: x.transpose(*d))(o, 0, 2, 1, 3).reshape(B, Sq, H * Dh) @ wo

    a = _A_ref(A_x, A_k_cache, A_v_cache, A_wq, A_wo)
    b = _B_ref(B_x, B_k_cache, B_v_cache, B_wq, B_wo)
    return jnp.concatenate([a, b], axis=-1)
```

```python
import functools, math
import numpy as np
import jax
import jax.numpy as jnp
import jax.experimental.pallas as pl
import jax.experimental.pallas.tpu as pltpu

B, SQ, D = 8, 144, 640
H, SK, DH = 32, 512, 128
M = B * SQ
KT = D // 128
U32, BF16, F32 = jnp.uint32, jnp.bfloat16, jnp.float32


def as_bf16(x):
    return pltpu.bitcast(x, BF16)


def _build(HG=4, NBUF=4, LA=4, RC=16, LAG=1, flags=None, nobounds=False, nodma=False, order="QAO", NQ=None, hoist=2, xb_at=None, wu32='', scopes=False):
    G = H // HG
    NSTEP = 2 * G
    NWQ = G
    if NQ is None:
        NQ = 8 if order == "QAO" else LA
    c_scale = float(DH ** -0.5 * math.log2(math.e))
    NT = (((1,), (1,)), ((), ()))

    def mod(u, n):
        if isinstance(u, int):
            return u % n
        if n & (n - 1) == 0:
            return jnp.bitwise_and(u, n - 1)
        return jax.lax.rem(u, n)

    def div(u, n):
        if isinstance(u, int):
            return u // n
        assert n & (n - 1) == 0
        return jnp.right_shift(u, int(math.log2(n)))

    def kernel(xa, ka, va, wqa, woa, xb, kb, vb, wqb, wob, out_ref,
               x_buf, k_buf, v_buf, wq_buf, wo_buf, q_scr, o_scr, acc_ref,
               sem_k, sem_v, sem_wq, sem_wo, sem_x):
        t = pl.program_id(0)
        x_h = (xa.bitcast(U32), xb.bitcast(U32)) if 'x' in wu32 else (xa, xb)
        k_h = (ka.bitcast(U32), kb.bitcast(U32))
        v_h = (va.bitcast(U32), vb.bitcast(U32))
        wq_h = (wqa.bitcast(U32), wqb.bitcast(U32)) if 'q' in wu32 else (wqa, wqb)
        wo_h = (woa.bitcast(U32), wob.bitcast(U32)) if 'o' in wu32 else (woa, wob)
        WOR = HG * DH // 2 if 'o' in wu32 else HG * DH
        ident = lambda z: z

        def cp_x(br):
            return pltpu.make_async_copy(x_h[br], x_buf.at[br], sem_x.at[br])

        def cp_k(br, g, slot):
            return pltpu.make_async_copy(k_h[br].at[:, pl.ds(g * HG, HG)], k_buf.at[slot], sem_k.at[slot])

        def cp_v(br, g, slot):
            return pltpu.make_async_copy(v_h[br].at[:, pl.ds(g * HG, HG)], v_buf.at[slot], sem_v.at[slot])

        def cp_wq(br, g, slot):
            return pltpu.make_async_copy(wq_h[br].at[:, pl.ds(g * (HG * DH), HG * DH)], wq_buf.at[slot], sem_wq.at[slot])

        def cp_wo(br, g, slot):
            return pltpu.make_async_copy(wo_h[br].at[pl.ds(g * WOR, WOR), :], wo_buf.at[slot], sem_wo.at[slot])

        def for_step(u, fn):
            if isinstance(u, int):
                if 0 <= u < NSTEP:
                    fn(u // G, u % G)
                return
            br_u = div(u, G)
            for br in range(2):
                @pl.when(br_u == br)
                def _():
                    fn(br, mod(u, G))

        def start_kvo(u):
            def fn(br, g):
                sl = mod(u, NBUF)
                cp_k(br, g, sl).start(); cp_v(br, g, sl).start(); cp_wo(br, g, sl).start()
            for_step(u, fn)

        def start_wq(u):
            for_step(u, lambda br, g: cp_wq(br, g, mod(u, NWQ)).start())

        def wait_on(buf, sem, slot):
            pltpu.make_async_copy(buf.at[slot], buf.at[slot], sem.at[slot]).wait()

        if not nodma:
            @pl.when(t == 0)
            def _():
                cp_x(0).start()
                for u in range(LA):
                    start_wq(u)
                for j in range(NBUF - 1):
                    start_kvo(j); start_wq(LA + j)
                if xb_at is None:
                    cp_x(1).start()
                if scopes:
                    with jax.named_scope("WAITX"):
                        cp_x(0).wait()
                else:
                    cp_x(0).wait()

        def prefetch(s):
            if nodma:
                return
            u = s + NBUF - 1
            start_kvo(u); start_wq(u + LA)

            if xb_at is not None:
                @pl.when(s == xb_at)
                def _():
                    cp_x(1).start()

        def waits(tq, s):
            if nodma:
                return
            if scopes:
                with jax.named_scope("WAITS"):
                    waits_(tq, s)
            else:
                waits_(tq, s)

        def waits_(tq, s):
            if s is not None:
                sl = mod(s, NBUF)
                wait_on(k_buf, sem_k, sl); wait_on(v_buf, sem_v, sl); wait_on(wo_buf, sem_wo, sl)
            if tq is not None:
                wait_on(wq_buf, sem_wq, mod(tq, NWQ))

                @pl.when(tq == G)
                def _():
                    cp_x(1).wait()

        def q_compute(u):
            x = (as_bf16 if 'x' in wu32 else ident)(x_buf[div(u, G)])
            wq = (as_bf16 if 'q' in wu32 else ident)(wq_buf[mod(u, NWQ)])
            return jnp.dot(x, wq, preferred_element_type=F32) * c_scale

        def q_store(u, q):
            qs = mod(u, NQ)
            for h in range(HG):
                q_scr[qs, h] = q[:, h * DH:(h + 1) * DH].astype(BF16)

        pairs = [(h, b) for h in range(HG) for b in range(B)]
        n = len(pairs)

        def att_fns(s):
            slot = mod(s, NBUF)
            qs = mod(s, NQ)

            def qk(i):
                h, b = pairs[i]
                qb = q_scr[qs, h, pl.ds(b * SQ, SQ)]
                kk = as_bf16(k_buf[slot, b, h])
                return jax.lax.dot_general(qb, kk, NT, preferred_element_type=F32)

            def softmax(sc):
                ps, rs = [], []
                for r in range(0, SQ, RC):
                    tt = sc[r:r + RC]
                    m = jnp.max(tt, axis=-1, keepdims=True)
                    p = jnp.exp2(tt - m)
                    l = jnp.sum(p, axis=-1, keepdims=True)
                    rc = pl.reciprocal(l, approx=True)
                    rc = rc * (2.0 - l * rc)
                    ps.append(p)
                    rs.append(rc)
                return jnp.concatenate(ps, axis=0).astype(BF16), rs

            def pv(i, p, rc):
                h, b = pairs[i]
                vv = as_bf16(v_buf[slot, b, h])
                o = jnp.dot(p, vv, preferred_element_type=F32)
                for ci, r in enumerate(range(0, SQ, RC)):
                    o_scr[h, pl.ds(b * SQ + r, RC)] = (o[r:r + RC] * rc[ci]).astype(BF16)
            return qk, softmax, pv

        def att_phase(s, mid=None, nhoist=0):
            qk, softmax, pv = att_fns(s)
            sc_q = {}
            nxt = 0
            if mid is not None:
                for i in range(nhoist):
                    sc_q[i] = qk(i)
                nxt = nhoist
                mid()
            done = 0
            while done < n:
                while nxt < n and nxt <= done + LAG and (nxt not in sc_q):
                    sc_q[nxt] = qk(nxt); nxt += 1
                p, rc = softmax(sc_q.pop(done))
                pv(done, p, rc)
                done += 1

        def o_phase(s):
            slot = mod(s, NBUF)
            first = mod(s, G) == 0
            o = jnp.concatenate([o_scr[h] for h in range(HG)], axis=1)
            wo = (as_bf16 if 'o' in wu32 else ident)(wo_buf[slot])
            acc = jnp.where(first, 0.0, acc_ref[...]) + jnp.dot(o, wo, preferred_element_type=F32)
            acc_ref[...] = acc
            out_ref[...] = acc.astype(out_ref.dtype)

        @pl.when(t < LA)
        def _():
            waits(t, None)
            q_store(t, q_compute(t))

        @pl.when(jnp.logical_and(t >= LA, t < NSTEP))
        def _():
            s = t - LA
            prefetch(s)
            waits(t, s)
            if order == "QAO":
                att_phase(s, mid=lambda: q_store(t, q_compute(t)), nhoist=hoist)
                o_phase(s)
            else:
                att_phase(s); o_phase(s); q_store(t, q_compute(t))

        @pl.when(t >= NSTEP)
        def _():
            s = t - LA
            prefetch(s)
            waits(None, s)
            att_phase(s); o_phase(s)

    def f(A_x, A_k_cache, A_v_cache, A_wq, A_wo, B_x, B_k_cache, B_v_cache, B_wq, B_wo):
        anyspec = pl.BlockSpec(memory_space=pl.ANY)
        out = pl.pallas_call(
            kernel,
            grid=(NSTEP + LA,),
            in_specs=[anyspec] * 10,
            out_specs=pl.BlockSpec((M, D), lambda t: (0, jnp.maximum(t - LA, 0) // G)),
            out_shape=jax.ShapeDtypeStruct((M, 2 * D), BF16),
            scratch_shapes=[
                pltpu.VMEM((2, M // 2, D), U32) if 'x' in wu32 else pltpu.VMEM((2, M, D), BF16),
                pltpu.VMEM((NBUF, B, HG, SK // 2, DH), U32),
                pltpu.VMEM((NBUF, B, HG, SK // 2, DH), U32),
                pltpu.VMEM((NWQ, D // 2, HG * DH), U32) if 'q' in wu32 else pltpu.VMEM((NWQ, D, HG * DH), BF16),
                pltpu.VMEM((NBUF, HG * DH // 2, D), U32) if 'o' in wu32 else pltpu.VMEM((NBUF, HG * DH, D), BF16),
                pltpu.VMEM((NQ, HG, M, DH), BF16),
                pltpu.VMEM((HG, M, DH), BF16),
                pltpu.VMEM((M, D), F32),
                pltpu.SemaphoreType.DMA((NBUF,)),
                pltpu.SemaphoreType.DMA((NBUF,)),
                pltpu.SemaphoreType.DMA((NWQ,)),
                pltpu.SemaphoreType.DMA((NBUF,)),
                pltpu.SemaphoreType.DMA((2,)),
            ],
            compiler_params=pltpu.CompilerParams(
                dimension_semantics=("arbitrary",),
                vmem_limit_bytes=110 * 1024 * 1024,
                flags=flags,
                disable_bounds_checks=nobounds,
            ),
        )(A_x.reshape(M, D), A_k_cache, A_v_cache, A_wq, A_wo,
          B_x.reshape(M, D), B_k_cache, B_v_cache, B_wq, B_wo)
        return out.reshape(B, SQ, 2 * D)
    return jax.jit(f)


def pallas_concat_heads__mha_block_cached__mha_block_cached__near_ridge_kernel(
    A_x, A_k_cache, A_v_cache, A_wq, A_wo, B_x, B_k_cache, B_v_cache, B_wq, B_wo):
    fn = _build(order="AOQ", nobounds=True, wu32="q")
    return fn(A_x, A_k_cache, A_v_cache, A_wq, A_wo, B_x, B_k_cache, B_v_cache, B_wq, B_wo)
```

```python
import math

import jax
import jax.numpy as jnp
import jax.experimental.pallas as pl
import jax.experimental.pallas.tpu as pltpu

B, SQ, D = 8, 144, 640
H, SK, DH = 32, 512, 128
M = B * SQ
MH = M // 2
HG = 4
G = H // HG
NSTEP = 2 * G
NBUF = 4
LA = 3
NQ = 4
NMAIN = NSTEP - LA
assert LA <= NBUF - 1 and LA < NQ
RC = 16
BF16, F32 = jnp.bfloat16, jnp.float32
C_SCALE = DH ** -0.5 * math.log2(math.e)
NT_DIMS = (((1,), (1,)), ((), ()))
QUADS = ((1, 1), (1, 0), (0, 0), (0, 1))
PAIRS = [(c * 2 + hh, r * 4 + bb) for (r, c) in QUADS for hh in range(2) for bb in range(4)]
NT = D // 128


def _mod(u, n):
    return u % n if isinstance(u, int) else jnp.bitwise_and(u, n - 1)


def _div(u, n):
    return u // n if isinstance(u, int) else jnp.right_shift(u, n.bit_length() - 1)


def _dot(a, b):
    return jnp.dot(a, b, preferred_element_type=F32)


def _kernel(xa, ka, va, wqa, woa, xb, kb, vb, wqb, wob, out_hbm,
            x_buf, kv_buf, wq_buf, wo_buf, q_scr, o_scr, acc_ref, out_stage,
            sem_kv, sem_wq, sem_wo, sem_xb, sem_out, sem_start, sem_order):
    kv_h = ((ka, kb), (va, vb))
    wq_h = (wqa, wqb)
    wo_h = (woa, wob)

    def keep_order():
        pl.semaphore_signal(sem_order, 1)
        pl.semaphore_wait(sem_order, 1)

    def kv_dst(which, slot, ci):
        r, c = QUADS[ci]
        return kv_buf.at[which, slot, pl.ds(r * 4, 4), pl.ds(c * 2, 2)]

    def start_kv(br, g, slot, ordered):
        for ci, (r, c) in enumerate(QUADS):
            for which in range(2):
                pltpu.make_async_copy(kv_h[which][br].at[pl.ds(r * 4, 4), pl.ds(g * HG + c * 2, 2)],
                                      kv_dst(which, slot, ci), sem_kv.at[which, slot, ci]).start()
            if ordered:
                keep_order()

    def wait_kv(slot, ci):
        for which in range(2):
            dst = kv_dst(which, slot, ci)
            pltpu.make_async_copy(dst, dst, sem_kv.at[which, slot, ci]).wait()

    def cp_wq(br, g):
        u = br * G + g
        return pltpu.make_async_copy(wq_h[br].at[:, pl.ds(g * (HG * DH), HG * DH)], wq_buf.at[u], sem_wq.at[u])

    def cp_wo(br, g):
        return pltpu.make_async_copy(wo_h[br].at[pl.ds(g * (HG * DH), HG * DH), :], wo_buf.at[g], sem_wo.at[g])

    def cp_xb():
        return pltpu.make_async_copy(xb, x_buf.at[1], sem_xb)

    def cp_out(br, r0, nr, c0, nc, si):
        return pltpu.make_async_copy(out_stage.at[br, pl.ds(r0, nr), pl.ds(c0, nc)],
                                     out_hbm.at[pl.ds(r0, nr), pl.ds(br * D + c0, nc)], sem_out.at[si])

    def wait_slot(buf, sem, slot):
        pltpu.make_async_copy(buf.at[slot], buf.at[slot], sem.at[slot]).wait()

    def per_branch(u, lo, hi, fn):
        for br in range(2):
            a, b = max(lo, br * G), min(hi, (br + 1) * G)
            if a < b:
                pl.when(jnp.logical_and(u >= a, u < b))(lambda br=br: fn(br))

    def prefetch(s):
        u = s + NBUF - 1
        lo, hi = NBUF - 1, NMAIN + NBUF - 1
        per_branch(u, lo, hi, lambda br: start_kv(br, _mod(u, G), _mod(u, NBUF), False))
        per_branch(u + 1, lo + 1, hi + 1, lambda br: cp_wo(br, _mod(u + 1, G)).start())
        w = u + LA + 1
        pl.when(w == G)(lambda: cp_xb().start())
        per_branch(w, lo + LA + 1, hi + LA + 1, lambda br: cp_wq(br, _mod(w, G)).start())

    def q_phase(u, stages=None):
        br = _div(u, G)
        qs = _mod(u, NQ)
        acc = [None, None]
        todo = [D, D]

        def part(r, c0, nc):
            v = _dot(x_buf[br, pl.ds(r * MH, MH), pl.ds(c0, nc)], wq_buf[u, pl.ds(c0, nc), :])
            acc[r] = v if acc[r] is None else acc[r] + v
            todo[r] -= nc
            if todo[r] == 0:
                q = acc[r] * C_SCALE
                for h in range(HG):
                    q_scr[qs, h, pl.ds(r * MH, MH)] = q[:, h * DH:(h + 1) * DH].astype(BF16)

        if stages is None:
            stages = [((), [(0, 0, D), (1, 0, D)])]
        for copies, items in stages:
            for cp in copies:
                cp.wait()
            for item in items:
                part(*item)

    def attend(s, lo, hi, before=None, after=None):
        slot = _mod(s, NBUF)
        qs = _mod(s, NQ)

        def scores(i):
            h, b = PAIRS[i]
            q = q_scr[qs, h, pl.ds(b * SQ, SQ)]
            k = kv_buf[0, slot, b, h]
            return jax.lax.dot_general(q, k, NT_DIMS, preferred_element_type=F32)

        def softmax(sc):
            ps, rs = [], []
            for r in range(0, SQ, RC):
                t = sc[r:r + RC]
                m = jnp.max(t, axis=-1, keepdims=True)
                p = jnp.exp2(t - m)
                l = jnp.sum(p, axis=-1, keepdims=True)
                rc = pltpu.reciprocal(l, approx=True)
                rc = rc * (2.0 - l * rc)
                ps.append(p)
                rs.append(rc)
            return jnp.concatenate(ps, axis=0).astype(BF16), rs

        def values(i, p, rs):
            h, b = PAIRS[i]
            o = _dot(p, kv_buf[1, slot, b, h])
            for ci, r in enumerate(range(0, SQ, RC)):
                o_scr[h, pl.ds(b * SQ + r, RC)] = (o[r:r + RC] * rs[ci]).astype(BF16)

        pending = {}
        for i in range(lo, hi + 1):
            if i < hi:
                if before and i in before:
                    before[i]()
                pending[i] = scores(i)
            if i > lo:
                values(i - 1, *softmax(pending.pop(i - 1)))
            if after and i in after:
                after[i]()

    def out_phase(s, r, br, done=None):
        g = _mod(s, G)
        first = g == 0
        rows = pl.ds(r * MH, MH)
        o = jnp.concatenate([o_scr[h, rows] for h in range(HG)], axis=1)
        for n in range(NT):
            cols = pl.ds(n * 128, 128)
            v = jnp.where(first, 0.0, acc_ref[rows, cols]) + _dot(o, wo_buf[g, :, cols])
            acc_ref[rows, cols] = v
            out_stage[br, rows, cols] = v.astype(BF16)
            if done is not None:
                done(r, n)

    def cp_x0(r, c0, nc, si):
        return pltpu.make_async_copy(xa.at[pl.ds(r * MH, MH), pl.ds(c0, nc)],
                                     x_buf.at[0, pl.ds(r * MH, MH), pl.ds(c0, nc)], sem_start.at[si])

    def cp_wq0(r0, nr, c0, nc, si):
        return pltpu.make_async_copy(wqa.at[pl.ds(r0, nr), pl.ds(c0, nc)],
                                     wq_buf.at[0, pl.ds(r0, nr), pl.ds(c0, nc)], sem_start.at[si])

    stages = [
        ([cp_wq0(0, 128, 0, 512, 0), cp_x0(0, 0, 128, 1)], [(0, 0, 128)]),
        ([cp_x0(1, 0, 128, 2)], [(1, 0, 128)]),
        ([cp_wq0(128, 128, 0, 512, 3), cp_x0(0, 128, 128, 4)], [(0, 128, 128)]),
        ([cp_x0(1, 128, 128, 5)], [(1, 128, 128)]),
        ([cp_wq0(256, 384, 0, 512, 6), cp_x0(0, 256, 384, 7)], [(0, 256, 384)]),
        ([cp_x0(1, 256, 384, 8)], [(1, 256, 384)]),
    ]
    for copies, _ in stages:
        for cp in copies:
            cp.start()
            keep_order()
    for u in range(1, LA + 1):
        cp_wq(0, u).start()
    keep_order()
    cp_wo(0, 0).start()
    for j in range(NBUF - 1):
        keep_order()
        start_kv(0, j, j, True)
        cp_wo(0, j + 1).start()
        cp_wq(0, LA + 1 + j).start()

    q_phase(0, stages)
    for u in range(1, LA):
        wait_slot(wq_buf, sem_wq, u)
        q_phase(u)

    def main_step(s, carry):
        slot = _mod(s, NBUF)
        wait_slot(wq_buf, sem_wq, s + LA)
        pl.when(s + LA == G)(lambda: cp_xb().wait())
        pl.when(s == G)(cp_out(0, 0, M, 0, D, 0).start)
        q_phase(s + LA)
        attend(s, 0, len(PAIRS),
               before={8 * ci: (lambda ci=ci: wait_kv(slot, ci)) for ci in range(4)},
               after={2: lambda: prefetch(s)})
        wait_slot(wo_buf, sem_wo, _mod(s, G))
        out_phase(s, 1, _div(s, G))
        out_phase(s, 0, _div(s, G))
        return carry

    jax.lax.fori_loop(0, NMAIN, main_step, 0)

    sent = []

    def last_steps(s, carry):
        is_last = s == NSTEP - 1
        slot = _mod(s, NBUF)

        def emit(r, n):
            desc = (1, r * MH, MH, n * 128, 128, len(sent) + 1)
            sent.append(desc)
            pl.when(is_last)(cp_out(*desc).start)

        wait_kv(slot, 0)
        attend(s, 0, 16, before={8: lambda: wait_kv(slot, 1)})
        wait_slot(wo_buf, sem_wo, _mod(s, G))
        wait_kv(slot, 2)
        attend(s, 16, 24)
        out_phase(s, 1, 1, emit)
        wait_kv(slot, 3)
        attend(s, 24, 32)
        out_phase(s, 0, 1, emit)
        return carry

    jax.lax.fori_loop(NMAIN, NSTEP, last_steps, 0)
    cp_out(0, 0, M, 0, D, 0).wait()
    for desc in sent:
        cp_out(*desc).wait()


@jax.jit
def pallas_concat_heads__mha_block_cached__mha_block_cached__near_ridge_kernel(
    A_x: jax.Array,
    A_k_cache: jax.Array,
    A_v_cache: jax.Array,
    A_wq: jax.Array,
    A_wo: jax.Array,
    B_x: jax.Array,
    B_k_cache: jax.Array,
    B_v_cache: jax.Array,
    B_wq: jax.Array,
    B_wo: jax.Array,
):
    hbm = pl.BlockSpec(memory_space=pl.ANY)
    out = pl.pallas_call(
        _kernel,
        in_specs=[hbm] * 10,
        out_specs=hbm,
        out_shape=jax.ShapeDtypeStruct((M, 2 * D), BF16),
        scratch_shapes=[
            pltpu.VMEM((2, M, D), BF16),
            pltpu.VMEM((2, NBUF, B, HG, SK, DH), BF16),
            pltpu.VMEM((NSTEP, D, HG * DH), BF16),
            pltpu.VMEM((G, HG * DH, D), BF16),
            pltpu.VMEM((NQ, HG, M, DH), BF16),
            pltpu.VMEM((HG, M, DH), BF16),
            pltpu.VMEM((M, D), F32),
            pltpu.VMEM((2, M, D), BF16),
            pltpu.SemaphoreType.DMA((2, NBUF, 4)),
            pltpu.SemaphoreType.DMA((NSTEP,)),
            pltpu.SemaphoreType.DMA((G,)),
            pltpu.SemaphoreType.DMA(()),
            pltpu.SemaphoreType.DMA((16,)),
            pltpu.SemaphoreType.DMA((9,)),
            pltpu.SemaphoreType.REGULAR,
        ],
        compiler_params=pltpu.CompilerParams(
            vmem_limit_bytes=100 * 1024 * 1024,
            flags={"XLA_TPU_RESCHEDULE_DMA_DONES": True},
            disable_bounds_checks=True,
            disable_semaphore_checks=True,
        ),
    )(A_x.reshape(M, D), A_k_cache, A_v_cache, A_wq, A_wo,
      B_x.reshape(M, D), B_k_cache, B_v_cache, B_wq, B_wo)
    return out.reshape(B, SQ, 2 * D)
```
